```python
import os as _os
_os.environ.setdefault('JAX_PLATFORMS', 'cpu')
import jax
import jax.numpy as jnp

def _softmax(x, axis=-1):
    return jax.nn.softmax(x, axis=axis)

def _gelu(x):
    return jax.nn.gelu(x, approximate=True)

def _silu(x):
    return jax.nn.silu(x)

def _sigmoid(x):
    return jax.nn.sigmoid(x)

def _layernorm(x, axis=-1, eps=1e-05):
    m = jnp.mean(x, axis=axis, keepdims=True)
    v = jnp.var(x, axis=axis, keepdims=True)
    return (x - m) / jnp.sqrt(v + eps)

def _scatter_add(tgt, idx, src, axis=0):
    return tgt.at[idx].add(src)

def _segment_sum(src, seg, n):
    return jax.ops.segment_sum(src, seg, n)

class _Rng:

    def __init__(self, key):
        self._k = key

    def _next(self):
        self._k, sub = jax.random.split(self._k)
        return sub

    def normal(self, shape):
        return jax.random.normal(self._next(), shape, dtype=jnp.bfloat16)

    def randint(self, lo, hi, shape):
        return jax.random.randint(self._next(), shape, lo, hi, dtype=jnp.int32)

    def uniform(self, shape, lo=0.0, hi=1.0):
        return jax.random.uniform(self._next(), shape, jnp.bfloat16, lo, hi)

    def permutation(self, n):
        return jax.random.permutation(self._next(), n)
kernel_name = 'standalone__conformer_conv_module__speech'

def setup_inputs():
    _rng = _Rng(jax.random.key(int.from_bytes(__import__("os").urandom(4), "little")))
    _w = lambda a: (lambda t: t.astype(jnp.bfloat16) if jnp.issubdtype(t.dtype, jnp.floating) else t)(jnp.asarray(a))
    B, T, D, K = (2, 16000, 256, 5)
    return {'x': _w((lambda *s: _rng.normal(s) * 0.2)(B, T, D)), 'w_pw1': _w((lambda *s: _rng.normal(s) * 0.2)(D, 2 * D)), 'dw': _w((lambda *s: _rng.normal(s) * 0.05)(K, D)), 'w_pw2': _w((lambda *s: _rng.normal(s) * 0.05)(D, D))}

def reference(x, w_pw1, dw, w_pw2):
    B, T, D = x.shape
    K = dw.shape[0]
    h = x @ w_pw1
    a, b = (h[..., :D].copy(), h[..., D:].copy())
    h = a * _sigmoid(b)
    pad = K // 2
    hp = jnp.pad(h, ((0, 0), (pad, pad), (0, 0)))
    out = jnp.zeros_like(h)
    for i in range(K):
        out = out + hp[:, i:i + T, :] * dw[i][None, None, :]
    return _silu(out) @ w_pw2
```

```python
import functools
import jax, jax.numpy as jnp
import numpy as np
from jax import lax
import jax.experimental.pallas as pl
import jax.experimental.pallas.tpu as pltpu


def make(BM=2000, pro=(256, 736), epi=(400, 800, 1200, 1600, 1872), vmem=110 * 2**20, flags=None, anchor=True,
         lowprio=1, nodma=False):
    D = 256
    H = 128
    SH = 16

    def kernel(x_hbm, w1_hbm, dw_hbm, w2_hbm, o_hbm, w1_ref, dw_ref, w2_ref, xb, ob, g_ref,
               xsem, psem, osem, esem, wsem, *, T, nB):
        R = nB * T
        N = R // BM

        def gpos(r):
            return 8 + r + 8 * (r // T)

        def xcopy(r0, n, sem):
            return pltpu.make_async_copy(x_hbm.at[pl.ds(r0, n)], xb.at[pl.ds(r0, n)], sem)

        def ocopy(r0, n, sem):
            return pltpu.make_async_copy(ob.at[pl.ds(r0, n)], o_hbm.at[pl.ds(r0, n)], sem)

        w1c = pltpu.make_async_copy(w1_hbm, w1_ref, wsem.at[0])
        dwc = pltpu.make_async_copy(dw_hbm, dw_ref, wsem.at[1])
        w2c = pltpu.make_async_copy(w2_hbm, w2_ref, wsem.at[2])

        cuts = [0] + list(pro) + [BM + SH]
        pieces = [(cuts[k], cuts[k + 1] - cuts[k]) for k in range(len(cuts) - 1)]
        pcopies = [xcopy(r0, n, psem.at[k]) for k, (r0, n) in enumerate(pieces)]

        def xchunk(i):
            r0 = i * BM + SH
            return xcopy(r0, min(BM, R - r0), xsem.at[i])

        w1c.start()
        pcopies[0].start()
        for c in pcopies[1:]:
            c.start(priority=lowprio)
        for i in range(1, N):
            xchunk(i).start(priority=lowprio)

        z = jnp.zeros((8, H), jnp.float32)
        for c in range(2):
            g_ref[c, 0:8, :] = z
            for b in range(nB):
                p = 8 + (b + 1) * T + 8 * b
                g_ref[c, p:p + 8, :] = z
        xb[R:R + SH, :] = jnp.zeros((SH, D), xb.dtype)

        def glu(a, b, segs):
            g = a + a * jnp.tanh(0.5 * b)
            o = 0
            for (m, dst) in segs:
                for c in range(2):
                    g_ref[c, pl.ds(dst, m), :] = g[o:o + m, c * H:(c + 1) * H]
                o += m

        def partA(r0, segs, between=None):
            n = sum(s[0] for s in segs)
            xs = xb[pl.ds(r0, n), :]
            a = jnp.dot(xs, w1_ref[:, :D], preferred_element_type=jnp.float32)
            if between is not None:
                between(a)
            b = jnp.dot(xs, w1_ref[:, D:], preferred_element_type=jnp.float32)
            glu(a, b, segs)

        def partB(dw, r0, n, gsrc, after=None):
            outs = []
            for c in range(2):
                acc = None
                for k in range(5):
                    t = g_ref[c, pl.ds(gsrc + (k - 2), n), :] * dw[k:k + 1, c * H:(c + 1) * H]
                    acc = t if acc is None else acc + t
                outs.append(acc + acc * jnp.tanh(acc))
            sv = jnp.concatenate(outs, axis=1).astype(jnp.bfloat16)
            o = jnp.dot(sv, w2_ref[...], preferred_element_type=jnp.float32)
            if after is None:
                ob[pl.ds(r0, n), :] = o.astype(ob.dtype)
            else:
                for (k0, m, f) in after:
                    ob[pl.ds(r0 + k0, m), :] = o[k0:k0 + m].astype(ob.dtype)
                    f()

        def xchunk_wait(i):
            r0 = pl.multiple_of(i * BM + SH, 16)

            @pl.when(i < N - 1)
            def _():
                xcopy(r0, BM, xsem.at[i]).wait()

            @pl.when(i == N - 1)
            def _():
                xcopy(r0, BM - SH, xsem.at[i]).wait()

        for k, (r0, n) in enumerate(pieces):
            pcopies[k].wait()
            if k == 0:
                w1c.wait()
                dwc.start()
                w2c.start()
            if r0 + n <= BM:
                partA(r0, [(n, gpos(r0))])
            else:
                partA(r0, [(BM - r0, gpos(r0)), (r0 + n - BM, gpos(BM))])
        dwc.wait()
        w2c.wait()
        dw = dw_ref[...].astype(jnp.float32) * 0.25

        def body(i, carry):
            xchunk_wait(i)
            rb = pl.multiple_of((i - 1) * BM, 16)
            partB(dw, rb, BM, gpos(rb))

            def between(a):
                ocopy(rb, BM, osem.at[i - 1]).start()
                if anchor:
                    ob[R:R + 16, :] = a[0:16, :].astype(ob.dtype)

            ra = pl.multiple_of(i * BM + SH, 16)
            rn = pl.multiple_of((i + 1) * BM, 16)
            partA(ra, [(BM - SH, pl.multiple_of(gpos(ra), 8)), (SH, pl.multiple_of(gpos(rn), 8))], between)
            return carry

        lax.fori_loop(1, N, body, 0)

        rb = (N - 1) * BM
        ec = [0] + list(epi) + [BM]
        ecopies = [ocopy(rb + ec[k], ec[k + 1] - ec[k], esem.at[k]) for k in range(len(ec) - 1)]
        partB(dw, rb, BM, gpos(rb), after=[(ec[k], ec[k + 1] - ec[k], ecopies[k].start) for k in range(len(ec) - 1)])
        for i in range(N - 1):
            ocopy(i * BM, BM, osem.at[i]).wait()
        for c in ecopies:
            c.wait()

    @jax.jit
    def fn(x, w_pw1, dw, w_pw2):
        B, T, D_ = x.shape
        R = B * T
        N = R // BM
        xf = x.reshape(R, D)
        out = pl.pallas_call(
            functools.partial(kernel, T=T, nB=B),
            in_specs=[pl.BlockSpec(memory_space=pl.ANY)] * 4,
            out_specs=pl.BlockSpec(memory_space=pl.ANY),
            out_shape=jax.ShapeDtypeStruct((R, D), x.dtype),
            scratch_shapes=[
                pltpu.VMEM(w_pw1.shape, w_pw1.dtype),
                pltpu.VMEM(dw.shape, dw.dtype),
                pltpu.VMEM(w_pw2.shape, w_pw2.dtype),
                pltpu.VMEM((R + SH, D), jnp.bfloat16),
                pltpu.VMEM((R + 16, D), jnp.bfloat16),
                pltpu.VMEM((2, R + 8 * (B + 1) + SH, H), jnp.float32),
                pltpu.SemaphoreType.DMA((N + 2,)),
                pltpu.SemaphoreType.DMA((len(pro) + 1,)),
                pltpu.SemaphoreType.DMA((N,)),
                pltpu.SemaphoreType.DMA((len(epi) + 1,)),
                pltpu.SemaphoreType.DMA((3,)),
            ],
            compiler_params=pltpu.CompilerParams(
                vmem_limit_bytes=vmem,
                flags=flags,
            ),
        )(xf, w_pw1, dw, w_pw2)
        return out.reshape(B, T, D)

    return fn


_fn = make(**dict(BM=4000, pro=(256,736,1936), epi=(800,1600,2400,3200,3600,3872)))


def pallas_standalone__conformer_conv_module__speech_kernel(
    x: jax.Array,
    w_pw1: jax.Array,
    dw: jax.Array,
    w_pw2: jax.Array,
):
    return _fn(x, w_pw1, dw, w_pw2)
```

```python
import functools

import jax
import jax.numpy as jnp
from jax import lax
import jax.experimental.pallas as pl
import jax.experimental.pallas.tpu as pltpu

_H = 128
_SH = 16
_PAD = 8

_RAMP = (256, 768, 2176, 4800)
_RAMP_SUB = 800
_WINDOWS = ((1600,) * 5, (1600, 1600, 528, 272))
_TAIL = (96, 96, 80)


def _split(n, sm, min_last=256):
    out = []
    while n > 0:
        k = min(sm, n)
        if 0 < n - k < min_last:
            k = n
        out.append(k)
        n -= k
    return out


def _kernel(x_hbm, w1_hbm, dw_hbm, w2_hbm, o_hbm,
            w1_ref, dw_ref, w2_ref, xb, ob, g_ref, xsem, psem, osem, *, T, nB):
    D = w2_ref.shape[0]
    K = dw_ref.shape[0]
    pad = K // 2
    ncol = D // _H
    R = nB * T
    R0 = sum(_RAMP)
    BM = sum(sum(w) for w in _WINDOWS)
    N = (R - R0) // BM
    assert pad <= _PAD and pad <= _SH and D % _H == 0
    assert R0 + N * BM == R
    ends = {R0}
    for i in range(N):
        p = R0 + i * BM
        for w in _WINDOWS:
            p += sum(w)
            ends.add(p)
    assert all(b * T in ends for b in range(1, nB + 1))

    def xcopy(r0, n, sem):
        return pltpu.make_async_copy(x_hbm.at[pl.ds(r0, n)], xb.at[pl.ds(r0, n)], sem)

    def ocopy(r0, n):
        return pltpu.make_async_copy(ob.at[pl.ds(r0, n)], o_hbm.at[pl.ds(r0, n)], osem)

    cuts = [0]
    for n in _RAMP:
        cuts.append(cuts[-1] + n)
    pcopies = []
    for k in range(len(_RAMP)):
        lo = 0 if k == 0 else cuts[k] + _SH
        hi = cuts[k + 1] + _SH
        pcopies.append(xcopy(lo, hi - lo, psem.at[k]))
    head = [
        pltpu.make_async_copy(w1_hbm, w1_ref, psem.at[0]),
        pcopies[0],
        pltpu.make_async_copy(dw_hbm, dw_ref, psem.at[0]),
        pltpu.make_async_copy(w2_hbm, w2_ref, psem.at[0]),
    ]
    for c in head:
        c.start()
    for c in pcopies[1:]:
        c.start(priority=1)
    for i in range(N):
        r0 = R0 + i * BM + _SH
        xcopy(r0, min(BM, R - r0), xsem.at[i]).start(priority=1)

    for c in range(ncol):
        g_ref[c, 0:_PAD, :] = jnp.zeros((_PAD, _H), jnp.float32)
    xb[R:R + _SH, :] = jnp.zeros((_SH, D), xb.dtype)

    def sub_block(dw, row0, o, n, first, last, keep, outs):
        lo = 0 if first else o + _SH
        m = o + n + _SH - lo
        xs = xb[pl.ds(row0 + lo, m), :]
        a = jnp.dot(xs, w1_ref[:, :D], preferred_element_type=jnp.float32)
        b = jnp.dot(xs, w1_ref[:, D:], preferred_element_type=jnp.float32)
        g = a + a * jnp.tanh(0.5 * b)
        for c in range(ncol):
            gc = g[:, c * _H:(c + 1) * _H]
            if not last:
                g_ref[c, _PAD + lo:_PAD + lo + m, :] = gc
            else:
                e = _PAD + lo + m - _SH
                g_ref[c, _PAD + lo:e, :] = gc[:m - _SH]
                g_ref[c, e:e + _PAD, :] = jnp.where(keep, gc[m - _SH:m - _SH + _PAD], 0.0)
        ss = []
        for c in range(ncol):
            acc = None
            for k in range(K):
                s0 = _PAD + o + k - pad
                t = g_ref[c, s0:s0 + n, :] * dw[k:k + 1, c * _H:(c + 1) * _H]
                acc = t if acc is None else acc + t
            ss.append(acc + acc * jnp.tanh(acc))
        sv = jnp.concatenate(ss, axis=1).astype(w2_ref.dtype)
        y = jnp.dot(sv, w2_ref[...], preferred_element_type=jnp.float32)
        if last:
            for c in range(ncol):
                gc = g[:, c * _H:(c + 1) * _H]
                g_ref[c, 0:_PAD, :] = jnp.where(keep, gc[m - _SH - _PAD:m - _SH], 0.0)
                g_ref[c, _PAD:_PAD + _SH, :] = gc[m - _SH:]
        p = 0
        for (k, emit) in outs:
            ob[pl.ds(row0 + o + p, k), :] = y[p:p + k].astype(ob.dtype)
            if emit is not None:
                emit(p, k)
            p += k

    def load_dw():
        return dw_ref[...].astype(jnp.float32) * 0.25

    def ramp():
        for k in range(len(_RAMP)):
            if k == 0:
                for c in head:
                    c.wait()
                dw = load_dw()
            else:
                pcopies[k].wait()
            o = cuts[k]
            for n in _split(_RAMP[k], _RAMP_SUB):
                sub_block(dw, 0, o, n, o == 0, o + n == R0, R0 % T != 0, [(n, None)])
                o += n
        ocopy(0, R0).start()

    def steady(i):
        r0 = pl.multiple_of(R0 + i * BM + _SH, 16)

        @pl.when(i < N - 1)
        def _():
            xcopy(r0, BM, xsem.at[i]).wait()

        @pl.when(i == N - 1)
        def _():
            xcopy(r0, BM - _SH, xsem.at[i]).wait()

        dw = load_dw()
        base = R0 + i * BM
        for wi, w in enumerate(_WINDOWS):
            row0 = pl.multiple_of(base, 16)
            keep = (base + sum(w)) % T != 0
            o = 0
            for s, n in enumerate(w):
                def emit(p, kk, o=o, row0=row0):
                    ocopy(pl.multiple_of(row0 + o + p, 16), kk).start()
                outs = [(n, emit)]
                if wi == len(_WINDOWS) - 1 and s == len(w) - 1:
                    outs = [(n - sum(_TAIL), emit)] if n > sum(_TAIL) else []
                    outs += [(t, emit) for t in _TAIL]
                sub_block(dw, row0, o, n, False, s == len(w) - 1, keep, outs)
                o += n
            base = base + sum(w)

    def body(j, carry):
        pl.when(j == 0)(ramp)
        pl.when(j > 0)(lambda: steady(j - 1))
        return carry

    lax.fori_loop(0, N + 1, body, 0)
    pltpu.make_async_copy(ob, o_hbm, osem).wait()


@jax.jit
def pallas_standalone__conformer_conv_module__speech_kernel(
    x: jax.Array,
    w_pw1: jax.Array,
    dw: jax.Array,
    w_pw2: jax.Array,
):
    B, T, D = x.shape
    R = B * T
    n_loop = (R - sum(_RAMP)) // sum(sum(w) for w in _WINDOWS)
    g_rows = max([sum(_RAMP)] + [sum(w) for w in _WINDOWS]) + _PAD + _SH
    out = pl.pallas_call(
        functools.partial(_kernel, T=T, nB=B),
        in_specs=[pl.BlockSpec(memory_space=pl.ANY)] * 4,
        out_specs=pl.BlockSpec(memory_space=pl.ANY),
        out_shape=jax.ShapeDtypeStruct((R, D), x.dtype),
        scratch_shapes=[
            pltpu.VMEM(w_pw1.shape, w_pw1.dtype),
            pltpu.VMEM(dw.shape, dw.dtype),
            pltpu.VMEM(w_pw2.shape, w_pw2.dtype),
            pltpu.VMEM((R + _SH, D), x.dtype),
            pltpu.VMEM((R, D), x.dtype),
            pltpu.VMEM((D // _H, g_rows, _H), jnp.float32),
            pltpu.SemaphoreType.DMA((n_loop,)),
            pltpu.SemaphoreType.DMA((len(_RAMP),)),
            pltpu.SemaphoreType.DMA(()),
        ],
        compiler_params=pltpu.CompilerParams(vmem_limit_bytes=110 * 2**20),
    )(x.reshape(R, D), w_pw1, dw, w_pw2)
    return out.reshape(B, T, D)
```
